```python
import jax
import jax.numpy as jnp

def _softmax(x, axis=-1):
    return jax.nn.softmax(x, axis=axis)
def _gelu(x):
    return jax.nn.gelu(x, approximate=True)
def _silu(x):
    return jax.nn.silu(x)
def _sigmoid(x):
    return jax.nn.sigmoid(x)
def _layernorm(x, axis=-1, eps=1e-5):
    m = jnp.mean(x, axis=axis, keepdims=True)
    v = jnp.var(x, axis=axis, keepdims=True)
    return (x - m) / jnp.sqrt(v + eps)
def _scatter_add(tgt, idx, src, axis=0):
    return tgt.at[idx].add(src)
def _segment_sum(src, seg, n):
    return jax.ops.segment_sum(src, seg, n)
class _Rng:
    def __init__(self, key):
        self._k = key
    def _next(self):
        self._k, sub = jax.random.split(self._k)
        return sub
    def normal(self, shape):
        return jax.random.normal(self._next(), shape, dtype=jnp.bfloat16)
    def randint(self, lo, hi, shape):
        return jax.random.randint(self._next(), shape, lo, hi, dtype=jnp.int32)
    def uniform(self, shape, lo=0.0, hi=1.0):
        return jax.random.uniform(self._next(), shape, jnp.bfloat16, lo, hi)
    def permutation(self, n):
        return jax.random.permutation(self._next(), n)


kernel_name = 'recurrent_scan__mha_block_cached__moe_arch_mod__decode'

def setup_inputs():
    _rng = _Rng(jax.random.key(int.from_bytes(__import__("os").urandom(4), "little")))
    _w = (lambda a: (lambda t: t.astype(jnp.bfloat16) if jnp.issubdtype(t.dtype, jnp.floating) else t)(jnp.asarray(a)))
    def _A_setup():
        B, Sq, D = 2, 1, 512
        H, Sk, Dh = 32, 16384, 128
        return {
            "x": _w((lambda *s: _rng.normal(s) * 0.05)(B, Sq, D)),
            "k_cache": _w((lambda *s: _rng.normal(s) * 0.05)(B, H, Sk, Dh)),
            "v_cache": _w((lambda *s: _rng.normal(s) * 0.05)(B, H, Sk, Dh)),
            "wq": _w((lambda *s: _rng.normal(s) * 0.05)(D, H * Dh) * (D ** -0.5)),
            "wo": _w((lambda *s: _rng.normal(s) * 0.05)(H * Dh, D) * ((H * Dh) ** -0.5)),
        }
    _A_in = _A_setup()

    def _B_setup():
        B, S, D, F, C = 2, 1, 512, 1792, 1
        return {
            "x": _w((lambda *s: _rng.normal(s) * 0.05)(B, S, D)),
            "w_r": _w((lambda *s: _rng.normal(s) * 0.05)(D)),
            "w_gate": _w((lambda *s: _rng.normal(s) * 0.05)(D, F)),
            "w_up": _w((lambda *s: _rng.normal(s) * 0.05)(D, F)),
            "w_down": _w((lambda *s: _rng.normal(s) * 0.05)(F, D)),
        }
    _B_in = _B_setup()

    return {
        "A_x": _A_in["x"],
        "A_k_cache": _A_in["k_cache"],
        "A_v_cache": _A_in["v_cache"],
        "A_wq": _A_in["wq"],
        "A_wo": _A_in["wo"],
        "B_x": _B_in["x"],
        "B_w_r": _B_in["w_r"],
        "B_w_gate": _B_in["w_gate"],
        "B_w_up": _B_in["w_up"],
        "B_w_down": _B_in["w_down"],
    }

def reference(A_x, A_k_cache, A_v_cache, A_wq, A_wo, B_x, B_w_r, B_w_gate, B_w_up, B_w_down):
    def _A_ref(x, k_cache, v_cache, wq, wo):
        B, Sq, D = x.shape
        H, Dh = 32, 128
        q = (lambda x, *d: x.transpose(*d))((x @ wq).reshape(B, Sq, H, Dh), 0, 2, 1, 3)
        scores = jnp.einsum("bhqd,bhkd->bhqk", q, k_cache) * (Dh ** -0.5)
        p = _softmax(scores, axis=-1)
        o = jnp.einsum("bhqk,bhkd->bhqd", p, v_cache)
        return (lambda x, *d: x.transpose(*d))(o, 0, 2, 1, 3).reshape(B, Sq, H * Dh) @ wo

    def _B_ref(x, w_r, w_gate, w_up, w_down):
        B, S, D = x.shape
        C = 1
        r = x @ w_r
        idx = jnp.argsort(-r, axis=-1)[:, :C]
        idx_e = jnp.repeat(idx.reshape(B, C, 1), D, axis=2)
        x_sel = jnp.take_along_axis(x, idx_e, axis=1)
        g = _silu(x_sel @ w_gate)
        u = x_sel @ w_up
        y = (g * u) @ w_down
        r_sel = _sigmoid(jnp.take_along_axis(r, idx, axis=1))
        y = y * r_sel.reshape(B, C, 1)
        b_off = (jnp.arange(B) * S).reshape(B, 1)
        flat_idx = (idx + b_off).reshape(B * C)
        zero = (x * 0.0).reshape(B * S, D)
        upd = _scatter_add(zero, flat_idx, y.reshape(B * C, D), axis=0)
        return x + upd.reshape(B, S, D)

    x = A_x
    xn = _layernorm(x, axis=-1)
    s = _A_ref(xn, A_k_cache, A_v_cache, A_wq, A_wo)
    g = _silu(_B_ref(xn, B_w_r, B_w_gate, B_w_up, B_w_down))
    return x + s * g
```

```python
import functools

import jax
import jax.numpy as jnp
import jax.experimental.pallas as pl
import jax.experimental.pallas.tpu as pltpu

_HEAD_DIM = 128
_ROWS = 8
_CHUNK = 2048
_PIECE = 128
_SLOTS = 4
_PIECE_ELEMS = _PIECE * _HEAD_DIM
_EPS = 1e-5

_F32 = jnp.float32
_BF16 = jnp.bfloat16


def _dot(a, b):
    return jnp.dot(a, b, preferred_element_type=_F32)


def _band_pieces(src, dst, r0, r1):
    cols = src.shape[1]
    rows = max(16, _PIECE_ELEMS // cols // 16 * 16)
    ncol = max(1, rows * cols // _PIECE_ELEMS)
    while cols % (ncol * 128):
        ncol -= 1
    width = cols // ncol
    out = []
    for r in range(r0, r1, rows):
        n = min(rows, r1 - r)
        for c in range(0, cols, width):
            idx = (pl.ds(r, n), pl.ds(c, width))
            out.append((src.at[idx], dst.at[idx]))
    return out


def _kernel(x_hbm, k_hbm, v_hbm, wq_hbm, wo_hbm, wr_hbm, wg_hbm, wu_hbm, wd_hbm,
            out_hbm,
            x_buf, wr_buf, wq_buf, wo_buf, wg_buf, wu_buf, wd_buf, k_buf, v_buf,
            q_scr, o_scr, gate_scr, out_buf, misc_sem, w_sem, kv_sem,
            *, heads, seq, chunk, piece, slots, wq_steps, wo_steps):
    batch, d_model = x_hbm.shape
    d_ff = wg_hbm.shape[1]
    chunks = seq // chunk
    n_kv = batch * heads * chunks
    scale = _HEAD_DIM ** -0.5

    def halves(src, dst, r0, r1):
        mid = (r0 + r1) // 2
        return [(src, dst, r0, mid), (src, dst, mid, r1)]

    wq_rows = d_model // wq_steps
    wo_rows = wo_hbm.shape[0] // wo_steps
    head_steps = [halves(wq_hbm, wq_buf, i * wq_rows, (i + 1) * wq_rows)
                  for i in range(wq_steps)]
    head_steps += [[(wg_hbm, wg_buf, r, r + d_model // 2), (wu_hbm, wu_buf, r, r + d_model // 2)]
                   for r in (0, d_model // 2)]
    head_steps += [halves(wd_hbm, wd_buf, 0, d_ff)]
    tail_steps = [halves(wo_hbm, wo_buf, i * wo_rows, (i + 1) * wo_rows)
                  for i in range(wo_steps)]
    n_head = len(head_steps)

    def start_weights(step, sem_idx):
        queues = [_band_pieces(*band) for band in step]
        for pair in zip(*queues, strict=True):
            for prio, (src, dst) in enumerate(pair):
                pltpu.make_async_copy(src, dst, w_sem.at[sem_idx, prio]).start(priority=prio)

    def wait_weights(step, sem_idx):
        for prio, (_, dst, r0, r1) in enumerate(step):
            band = dst.at[pl.ds(r0, r1 - r0)]
            pltpu.make_async_copy(band, band, w_sem.at[sem_idx, prio]).wait()

    def start_kv(step, slot):
        for r in range(0, chunk, piece):
            src = pl.ds(pl.multiple_of(step * chunk + r, piece), piece)
            for prio, (hbm, buf) in enumerate(((k_hbm, k_buf), (v_hbm, v_buf))):
                pltpu.make_async_copy(hbm.at[src], buf.at[slot, pl.ds(r, piece)],
                                      kv_sem.at[prio, slot]).start(priority=prio)

    def wait_kv(buf, which, slot):
        pltpu.make_async_copy(buf.at[slot], buf.at[slot], kv_sem.at[which, slot]).wait()

    def start_prologue(i):
        if i < n_head:
            start_weights(head_steps[i], i)
        else:
            start_kv(i - n_head, i - n_head)

    x_copy = pltpu.make_async_copy(x_hbm, x_buf, misc_sem.at[0])
    wr_copy = pltpu.make_async_copy(wr_hbm, wr_buf, misc_sem.at[1])
    x_copy.start(priority=0)
    wr_copy.start(priority=1)
    issued = 0

    def issue_one():
        nonlocal issued
        start_prologue(issued)
        issued += 1

    issue_one()
    x_copy.wait()
    wr_copy.wait()

    x = jnp.concatenate([x_buf[...].astype(_F32),
                         jnp.zeros((_ROWS - batch, d_model), _F32)], axis=0)
    mean = jnp.mean(x, axis=-1, keepdims=True)
    cent = x - mean
    var = jnp.mean(cent * cent, axis=-1, keepdims=True)
    xn_b = (cent / jnp.sqrt(var + _EPS)).astype(_BF16)
    xn = xn_b.astype(_F32)
    for _ in range(slots - 1):
        issue_one()

    q = None
    for i in range(wq_steps):
        wait_weights(head_steps[i], i)
        rows = slice(i * wq_rows, (i + 1) * wq_rows)
        part = _dot(xn_b[:, rows], wq_buf[rows, :])
        q = part if q is None else q + part
        issue_one()
    for h in range(heads):
        q_scr[h] = q[:, h * _HEAD_DIM:(h + 1) * _HEAD_DIM]

    gate = up = None
    for i in range(2):
        wait_weights(head_steps[wq_steps + i], wq_steps + i)
        rows = slice(i * d_model // 2, (i + 1) * d_model // 2)
        g_part = _dot(xn_b[:, rows], wg_buf[rows, :])
        u_part = _dot(xn_b[:, rows], wu_buf[rows, :])
        gate = g_part if gate is None else gate + g_part
        up = u_part if up is None else up + u_part
        issue_one()
    hidden = (jax.nn.silu(gate) * up).astype(_BF16)
    wait_weights(head_steps[-1], n_head - 1)
    y = _dot(hidden, wd_buf[...])
    issue_one()
    route = jnp.sum(xn * wr_buf[...].astype(_F32).reshape(1, d_model), axis=-1, keepdims=True)
    routed = xn + (xn * 0.0 + y * jax.nn.sigmoid(route))
    gate_scr[...] = jax.nn.silu(routed)
    o_scr[...] = jnp.zeros(o_scr.shape, _F32)

    row = jax.lax.broadcasted_iota(jnp.int32, (_ROWS, _HEAD_DIM), 0)

    def head_body(bh, _):
        b = bh // heads
        h = bh % heads
        q_h = q_scr[h].astype(_BF16)

        def chunk_body(c, carry):
            m_prev, l_prev, acc = carry
            step = bh * chunks + c
            slot = step % slots
            wait_kv(k_buf, 0, slot)
            wait_kv(v_buf, 1, slot)
            s = jax.lax.dot_general(q_h, k_buf[slot], (((1,), (1,)), ((), ())),
                                    preferred_element_type=_F32) * scale
            cols = [s[:, i:i + 128] for i in range(0, chunk, 128)]
            m_new = jnp.maximum(
                m_prev, jnp.max(functools.reduce(jnp.maximum, cols), axis=-1, keepdims=True))
            alpha = jnp.exp(m_prev - m_new)
            p_cols = [jnp.exp(col - m_new) for col in cols]
            l_new = alpha * l_prev + functools.reduce(jnp.add, p_cols)
            p = jnp.concatenate(p_cols, axis=-1).astype(_BF16)
            acc = alpha * acc + _dot(p, v_buf[slot])

            nxt = step + slots

            @pl.when(nxt < n_kv)
            def _():
                start_kv(nxt, slot)

            @pl.when(nxt >= n_kv)
            def _():
                for i in range(min(slots, wo_steps)):
                    pl.when(nxt == n_kv + i)(
                        functools.partial(start_weights, tail_steps[i], n_head + i))

            return m_new, l_new, acc

        init = (jnp.full((_ROWS, _HEAD_DIM), -jnp.inf, _F32),
                jnp.zeros((_ROWS, _HEAD_DIM), _F32),
                jnp.zeros((_ROWS, _HEAD_DIM), _F32))
        _, l, acc = jax.lax.fori_loop(0, chunks, chunk_body, init)
        o = acc / jnp.sum(l, axis=-1, keepdims=True)
        o_scr[h] = jnp.where(row == b, o, o_scr[h])

    jax.lax.fori_loop(0, batch * heads, head_body, None)

    s = None
    heads_per_step = heads // wo_steps
    for i in range(wo_steps):
        if i + slots < wo_steps:
            start_weights(tail_steps[i + slots], n_head + i + slots)
        wait_weights(tail_steps[i], n_head + i)
        o = jnp.concatenate([o_scr[i * heads_per_step + j] for j in range(heads_per_step)],
                            axis=-1).astype(_BF16)
        part = _dot(o, wo_buf[i * wo_rows:(i + 1) * wo_rows, :])
        s = part if s is None else s + part
    out_buf[...] = (x_buf[...].astype(_F32) + (s * gate_scr[...])[:batch]).astype(out_buf.dtype)
    out_copy = pltpu.make_async_copy(out_buf, out_hbm, misc_sem.at[0])
    out_copy.start()
    out_copy.wait()


def _call(x, k, v, wq, wo, wr, wg, wu, wd, *, chunk=_CHUNK, piece=_PIECE, slots=_SLOTS,
          wq_steps=4, wo_steps=4, **params):
    batch, heads, seq, head_dim = k.shape
    d_model = x.shape[-1]
    assert head_dim == _HEAD_DIM and x.shape[1] == 1 and batch <= _ROWS
    assert seq % chunk == 0 and chunk % piece == 0
    n_weight_steps = wq_steps + 3 + wo_steps
    hbm = pl.BlockSpec(memory_space=pltpu.HBM)
    out = pl.pallas_call(
        functools.partial(_kernel, heads=heads, seq=seq, chunk=chunk, piece=piece, slots=slots,
                          wq_steps=wq_steps, wo_steps=wo_steps),
        in_specs=[hbm] * 9,
        out_specs=hbm,
        out_shape=jax.ShapeDtypeStruct((batch, d_model), x.dtype),
        scratch_shapes=[
            pltpu.VMEM((batch, d_model), x.dtype),
            pltpu.VMEM(wr.shape, wr.dtype),
            pltpu.VMEM(wq.shape, wq.dtype),
            pltpu.VMEM(wo.shape, wo.dtype),
            pltpu.VMEM(wg.shape, wg.dtype),
            pltpu.VMEM(wu.shape, wu.dtype),
            pltpu.VMEM(wd.shape, wd.dtype),
            pltpu.VMEM((slots, chunk, head_dim), k.dtype),
            pltpu.VMEM((slots, chunk, head_dim), v.dtype),
            pltpu.VMEM((heads, _ROWS, head_dim), _F32),
            pltpu.VMEM((heads, _ROWS, head_dim), _F32),
            pltpu.VMEM((_ROWS, d_model), _F32),
            pltpu.VMEM((batch, d_model), x.dtype),
            pltpu.SemaphoreType.DMA((2,)),
            pltpu.SemaphoreType.DMA((n_weight_steps, 2)),
            pltpu.SemaphoreType.DMA((2, slots)),
        ],
        compiler_params=pltpu.CompilerParams(vmem_limit_bytes=64 * 1024 * 1024, **params),
    )(x.reshape(batch, d_model), k.reshape(-1, head_dim), v.reshape(-1, head_dim),
      wq, wo, wr, wg, wu, wd)
    return out.reshape(x.shape)


@jax.jit
def pallas_recurrent_scan__mha_block_cached__moe_arch_mod__decode_kernel(
    A_x: jax.Array,
    A_k_cache: jax.Array,
    A_v_cache: jax.Array,
    A_wq: jax.Array,
    A_wo: jax.Array,
    B_x: jax.Array,
    B_w_r: jax.Array,
    B_w_gate: jax.Array,
    B_w_up: jax.Array,
    B_w_down: jax.Array,
):
    del B_x
    return _call(A_x, A_k_cache, A_v_cache, A_wq, A_wo, B_w_r, B_w_gate, B_w_up, B_w_down)
```

```python
import functools

import jax
import jax.numpy as jnp
import jax.experimental.pallas as pl
import jax.experimental.pallas.tpu as pltpu

_HEAD_DIM = 128
_ROWS = 8
_IN_FLIGHT = 64
_EPS = 1e-5

_F32 = jnp.float32
_BF16 = jnp.bfloat16


def _dot(a, b):
    return jnp.dot(a, b, preferred_element_type=_F32)


def _tiles(r0, r1, rows, cols, width):
    return [(pl.ds(r, rows), pl.ds(c, width))
            for r in range(r0, r1, rows) for c in range(0, cols, width)]


def _interleave(streams):
    return [item for group in zip(*streams, strict=True) for item in group]


def _copies(src, dst, sem, streams):
    return [(src.at[idx], dst.at[idx], sem) for idx in _interleave(streams)]


def _wait_all(buf, sem):
    pltpu.make_async_copy(buf, buf, sem).wait()


def _kernel(x_hbm, k_hbm, v_hbm, wq_hbm, wo_hbm, wr_hbm, wg_hbm, wu_hbm, wd_hbm,
            out_hbm,
            kv_buf, wq_buf, wo_buf, ff_buf, wd_buf, x_buf, wr_buf,
            q_scr, o_scr, gate_scr, out_buf, sem, wo_sem, kv_sem,
            *, heads, seq, chunk, tile, piece, run, streams, slots, wo_groups, split):
    batch, d_model = x_hbm.shape
    d_ff = wg_hbm.shape[1]
    d_attn = heads * _HEAD_DIM
    chunks = seq // chunk
    n_kv = batch * heads * chunks
    ahead = slots - 1
    scale = _HEAD_DIM ** -0.5
    x_sem, wr_sem, wq_sem, ff_sem, wd_sem = (sem.at[i] for i in range(5))

    def kv_copies(step, slot):
        base = (step // chunks) * seq + (step % chunks) * (chunk // streams)
        out = []
        for first in range(0, chunk // piece, run):
            for which, hbm in enumerate((k_hbm, v_hbm)):
                for i in range(first, first + run):
                    row = base + (i % streams) * (seq // streams) + (i // streams) * piece
                    if not isinstance(row, int):
                        row = pl.multiple_of(row, piece)
                    out.append((hbm.at[pl.ds(row, piece)],
                                kv_buf.at[slot, which, pl.ds(i * piece, piece)], kv_sem.at[slot]))
        return out

    def with_queues(copies, run):
        return [(copy, i // run % 2) for i, copy in enumerate(copies)]

    def spread(copies, n):
        units = len(copies) // 4
        done = 0
        for i in range(n):
            yield i
            upto = len(copies) if i == n - 1 else units * (i + 1) // n * 4
            for copy, queue in copies[done:upto]:
                pltpu.make_async_copy(*copy).start(priority=queue)
            done = upto

    def start(copies):
        for _ in spread(copies, 1):
            pass

    def bands(n_rows, n, *tile):
        return [_tiles(i * n_rows // n, (i + 1) * n_rows // n, *tile) for i in range(n)]

    wq_copies = _copies(wq_hbm, wq_buf, wq_sem, bands(d_model, 8, 8, d_attn, 1024))
    ff_copies = _interleave([
        _copies(wg_hbm, ff_buf.at[0], ff_sem, bands(d_model, 4, 8, d_ff, d_ff)),
        _copies(wu_hbm, ff_buf.at[1], ff_sem, bands(d_model, 4, 8, d_ff, d_ff))])
    wd_copies = _copies(wd_hbm, wd_buf, wd_sem, bands(d_ff, 4, 16, d_model, d_model))
    pending = with_queues(wq_copies, 2) + with_queues(ff_copies, 1) + with_queues(wd_copies, 2)
    for step in range(ahead):
        pending += with_queues(kv_copies(step, step), run)
    wq_done = len(wq_copies) + _IN_FLIGHT
    ff_done = wq_done + len(ff_copies)
    wd_done = ff_done + len(wd_copies)

    start(with_queues([(x_hbm, x_buf, x_sem), (wr_hbm, wr_buf, wr_sem)], 1))
    start(pending[:_IN_FLIGHT])
    _wait_all(x_buf, x_sem)
    _wait_all(wr_buf, wr_sem)
    x = jnp.concatenate([x_buf[...].astype(_F32),
                         jnp.zeros((_ROWS - batch, d_model), _F32)], axis=0)
    cent = x - jnp.mean(x, axis=-1, keepdims=True)
    var = jnp.mean(cent * cent, axis=-1, keepdims=True)
    xn_b = (cent / jnp.sqrt(var + _EPS)).astype(_BF16)
    xn = xn_b.astype(_F32)
    route = jnp.sum(xn * wr_buf[...].astype(_F32).reshape(1, d_model), axis=-1, keepdims=True)
    o_scr[...] = jnp.zeros(o_scr.shape, _F32)
    start(pending[_IN_FLIGHT:wq_done])

    _wait_all(wq_buf, wq_sem)
    for h in spread(pending[wq_done:ff_done], heads):
        q_scr[h] = _dot(xn_b, wq_buf[:, h * _HEAD_DIM:(h + 1) * _HEAD_DIM])

    _wait_all(ff_buf, ff_sem)
    hidden = []
    for i in spread(pending[ff_done:wd_done], d_ff // 128):
        cols = slice(i * 128, (i + 1) * 128)
        hidden.append((jax.nn.silu(_dot(xn_b, ff_buf[0, :, cols]))
                       * _dot(xn_b, ff_buf[1, :, cols])).astype(_BF16))

    _wait_all(wd_buf, wd_sem)
    y = 0.0
    for i in spread(pending[wd_done:], d_ff // 128):
        y = y + _dot(hidden[i], wd_buf[i * 128:(i + 1) * 128, :])
    gate_scr[...] = jax.nn.silu(xn + (xn * 0.0 + y * jax.nn.sigmoid(route)))

    row = jax.lax.broadcasted_iota(jnp.int32, (_ROWS, _HEAD_DIM), 0)

    def attend(step, carry, copies):
        b, h, c = step // (heads * chunks), step // chunks % heads, step % chunks
        slot = step % slots
        m_prev, l_prev, acc = carry
        q = q_scr[h].astype(_BF16)
        n = chunk // tile
        half = len(copies) * split // 16 * 4
        _wait_all(kv_buf.at[slot], kv_sem.at[slot])
        cols = []
        for i in spread(copies[:half], n):
            s = jax.lax.dot_general(q, kv_buf[slot, 0, i * tile:(i + 1) * tile, :],
                                    (((1,), (1,)), ((), ())), preferred_element_type=_F32) * scale
            cols += [s[:, j:j + 128] for j in range(0, tile, 128)]
        m_new = jnp.maximum(
            m_prev, jnp.max(functools.reduce(jnp.maximum, cols), axis=-1, keepdims=True))
        alpha = jnp.exp(m_prev - m_new)
        p_cols = [jnp.exp(col - m_new) for col in cols]
        l_new = alpha * l_prev + functools.reduce(jnp.add, p_cols)
        acc = alpha * acc
        for i in spread(copies[half:], n):
            p = jnp.concatenate(p_cols[i * tile // 128:(i + 1) * tile // 128], axis=-1)
            acc = acc + _dot(p.astype(_BF16), kv_buf[slot, 1, i * tile:(i + 1) * tile, :])

        last = c == chunks - 1

        @pl.when(last)
        def _():
            o = acc / jnp.sum(l_new, axis=-1, keepdims=True)
            o_scr[h] = jnp.where(row == b, o, o_scr[h])

        return (jnp.where(last, -jnp.inf, m_new), jnp.where(last, 0.0, l_new),
                jnp.where(last, 0.0, acc))

    def main_step(step, carry):
        nxt = step + ahead
        return attend(step, carry, with_queues(kv_copies(nxt, nxt % slots), run))

    carry = (jnp.full((_ROWS, _HEAD_DIM), -jnp.inf, _F32),
             jnp.zeros((_ROWS, _HEAD_DIM), _F32),
             jnp.zeros((_ROWS, _HEAD_DIM), _F32))
    carry = jax.lax.fori_loop(0, n_kv - ahead, main_step, carry)

    order = [h for i in range(4) for h in range(i, heads, 4)]
    groups, wo_copies = [], []
    for g, size in enumerate(wo_groups):
        group, order = order[:size], order[size:]
        groups.append(group)
        wo_copies += _copies(wo_hbm, wo_buf, wo_sem.at[g], [
            _tiles(h * _HEAD_DIM, (h + 1) * _HEAD_DIM, 16, d_model, d_model) for h in group])
    assert not order
    pending = with_queues(wo_copies, 2)
    per_step = 2 * chunk // piece
    for step in range(n_kv - ahead, n_kv):
        carry = attend(step, carry, pending[:per_step])
        pending = pending[per_step:]

    s = 0.0
    for g, group in enumerate(groups):
        _wait_all(wo_buf.at[pl.ds(0, len(group) * _HEAD_DIM)], wo_sem.at[g])
        for i in spread(pending, len(group)):
            h = group[i]
            s = s + _dot(o_scr[h].astype(_BF16), wo_buf[h * _HEAD_DIM:(h + 1) * _HEAD_DIM, :])
        pending = []
    out_buf[...] = (x_buf[...].astype(_F32) + (s * gate_scr[...])[:batch]).astype(out_buf.dtype)
    out_copy = pltpu.make_async_copy(out_buf, out_hbm, x_sem)
    out_copy.start()
    out_copy.wait()


def _call(x, k, v, wq, wo, wr, wg, wu, wd, *, chunk=2048, tile=256, piece=64, run=2, streams=8, slots=4,
          wo_groups=(8, 8, 8, 4, 2, 2), split=2, **params):
    batch, heads, seq, head_dim = k.shape
    d_model = x.shape[-1]
    assert head_dim == _HEAD_DIM and x.shape[1] == 1 and batch <= _ROWS
    assert seq % chunk == 0 and chunk % (piece * streams) == 0 and chunk % (piece * run) == 0
    hbm = pl.BlockSpec(memory_space=pltpu.HBM)
    out = pl.pallas_call(
        functools.partial(_kernel, heads=heads, seq=seq, chunk=chunk, tile=tile, piece=piece, run=run,
                          streams=streams, slots=slots, wo_groups=wo_groups, split=split),
        in_specs=[hbm] * 9,
        out_specs=hbm,
        out_shape=jax.ShapeDtypeStruct((batch, d_model), x.dtype),
        scratch_shapes=[
            pltpu.VMEM((slots, 2, chunk, head_dim), k.dtype),
            pltpu.VMEM(wq.shape, wq.dtype),
            pltpu.VMEM(wo.shape, wo.dtype),
            pltpu.VMEM((2,) + wg.shape, wg.dtype),
            pltpu.VMEM(wd.shape, wd.dtype),
            pltpu.VMEM((batch, d_model), x.dtype),
            pltpu.VMEM(wr.shape, wr.dtype),
            pltpu.VMEM((heads, _ROWS, head_dim), _F32),
            pltpu.VMEM((heads, _ROWS, head_dim), _F32),
            pltpu.VMEM((_ROWS, d_model), _F32),
            pltpu.VMEM((batch, d_model), x.dtype),
            pltpu.SemaphoreType.DMA((5,)),
            pltpu.SemaphoreType.DMA((len(wo_groups),)),
            pltpu.SemaphoreType.DMA((slots,)),
        ],
        compiler_params=pltpu.CompilerParams(vmem_limit_bytes=64 * 1024 * 1024, **params),
    )(x.reshape(batch, d_model), k.reshape(-1, head_dim), v.reshape(-1, head_dim),
      wq, wo, wr, wg, wu, wd)
    return out.reshape(x.shape)


@jax.jit
def pallas_recurrent_scan__mha_block_cached__moe_arch_mod__decode_kernel(
    A_x: jax.Array,
    A_k_cache: jax.Array,
    A_v_cache: jax.Array,
    A_wq: jax.Array,
    A_wo: jax.Array,
    B_x: jax.Array,
    B_w_r: jax.Array,
    B_w_gate: jax.Array,
    B_w_up: jax.Array,
    B_w_down: jax.Array,
):
    del B_x
    return _call(A_x, A_k_cache, A_v_cache, A_wq, A_wo, B_w_r, B_w_gate, B_w_up, B_w_down)
```

```python
import functools

import jax
import jax.numpy as jnp
import jax.experimental.pallas as pl
import jax.experimental.pallas.tpu as pltpu

_HEAD_DIM = 128
_GROUP = 8
_IN_FLIGHT = 64
_EPS = 1e-5

_F32 = jnp.float32
_BF16 = jnp.bfloat16


def _dot(a, b):
    return jnp.dot(a, b, preferred_element_type=_F32)


def _tiles(r0, r1, rows, cols, width):
    return [(pl.ds(r, rows), pl.ds(c, width))
            for r in range(r0, r1, rows) for c in range(0, cols, width)]


def _bands(n_rows, n, *tile):
    return [_tiles(i * n_rows // n, (i + 1) * n_rows // n, *tile) for i in range(n)]


def _interleave(streams):
    return [item for group in zip(*streams, strict=True) for item in group]


def _copies(src, dst, sem, streams):
    return [(src.at[idx], dst.at[idx], sem) for idx in _interleave(streams)]


def _with_queues(copies, run):
    return [(copy, i // run % 2) for i, copy in enumerate(copies)]


def _start(copies):
    for copy, queue in copies:
        pltpu.make_async_copy(*copy).start(priority=queue)


def _spread(copies, n):
    done = 0
    for i in range(n):
        yield i
        upto = len(copies) if i == n - 1 else len(copies) // 4 * (i + 1) // n * 4
        _start(copies[done:upto])
        done = upto


def _wait_all(buf, sem):
    pltpu.make_async_copy(buf, buf, sem).wait()


def _kernel(x_hbm, k_hbm, v_hbm, wq_hbm, wo_hbm, wr_hbm, wg_hbm, wu_hbm, wd_hbm,
            out_hbm,
            kv_buf, wq_buf, wo_buf, ff_buf, wd_buf, x_buf, wr_buf,
            q_scr, o_scr, gate_scr, out_buf, sem, wo_sem, kv_sem,
            *, heads, seq, keys, piece, stride, slots, wo_groups):
    batch, d_model = x_hbm.shape
    d_ff = wg_hbm.shape[1]
    groups = heads // _GROUP
    chunks = seq // keys
    n_kv = batch * groups * chunks
    ahead = slots - 1
    scale = _HEAD_DIM ** -0.5
    x_sem, wr_sem, wq_sem, ff_sem, wd_sem = (sem.at[i] for i in range(5))

    def head_of(g, j):
        return g // stride * (stride * _GROUP) + g % stride + j * stride

    def split(step):
        return step // (groups * chunks), step // chunks % groups, step % chunks

    def kv_copies(step, slot):
        b, g, c = split(step)
        base = (b * heads + head_of(g, 0)) * seq + c * keys
        copies = []
        for r in range(0, keys, piece):
            for first in range(0, _GROUP, 2):
                for which, hbm in enumerate((k_hbm, v_hbm)):
                    for j in (first, first + 1):
                        src = base + head_of(0, j) * seq + r
                        if not isinstance(src, int):
                            src = pl.multiple_of(src, piece)
                        copies.append((hbm.at[pl.ds(src, piece)],
                                       kv_buf.at[slot, which, j, pl.ds(r, piece)],
                                       kv_sem.at[slot]))
        return _with_queues(copies, 2)

    def sublane(rows, cols):
        return jax.lax.broadcasted_iota(jnp.int32, (rows, cols), 0) % _GROUP

    wq_copies = _copies(wq_hbm, wq_buf, wq_sem, _bands(d_model, 8, 8, wq_hbm.shape[1], 1024))
    ff_copies = _interleave([
        _copies(wg_hbm, ff_buf.at[0], ff_sem, _bands(d_model, 4, 8, d_ff, d_ff)),
        _copies(wu_hbm, ff_buf.at[1], ff_sem, _bands(d_model, 4, 8, d_ff, d_ff))])
    wd_copies = _copies(wd_hbm, wd_buf, wd_sem, _bands(d_ff, 4, 16, d_model, d_model))
    pending = _with_queues(wq_copies, 2) + _with_queues(ff_copies, 1) + _with_queues(wd_copies, 2)
    for step in range(ahead):
        pending += kv_copies(step, step)
    wq_done = len(wq_copies) + _IN_FLIGHT
    ff_done = wq_done + len(ff_copies)
    wd_done = ff_done + len(wd_copies)

    _start(_with_queues([(x_hbm, x_buf, x_sem), (wr_hbm, wr_buf, wr_sem)], 1))
    _start(pending[:_IN_FLIGHT])
    _wait_all(x_buf, x_sem)
    _wait_all(wr_buf, wr_sem)
    x = x_buf[...].astype(_F32)
    x = jnp.concatenate(
        [jnp.broadcast_to(x[b:b + 1], (_GROUP, d_model)) for b in range(batch)], axis=0)
    cent = x - jnp.mean(x, axis=-1, keepdims=True)
    var = jnp.mean(cent * cent, axis=-1, keepdims=True)
    xn_b = (cent / jnp.sqrt(var + _EPS)).astype(_BF16)
    xn = xn_b.astype(_F32)
    route = jnp.sum(xn * wr_buf[...].astype(_F32).reshape(1, d_model), axis=-1, keepdims=True)
    _start(pending[_IN_FLIGHT:wq_done])

    _wait_all(wq_buf, wq_sem)
    lane_rows = sublane(batch * _GROUP, _HEAD_DIM)
    for i in _spread(pending[wq_done:ff_done], heads):
        g, j = divmod(i, _GROUP)
        h = head_of(g, j)
        q_h = _dot(xn_b, wq_buf[:, h * _HEAD_DIM:(h + 1) * _HEAD_DIM])
        q = q_h if j == 0 else jnp.where(lane_rows == j, q_h, q)
        if j == _GROUP - 1:
            q_scr[g] = q

    _wait_all(ff_buf, ff_sem)
    hidden = []
    for i in _spread(pending[ff_done:wd_done], d_ff // 128):
        cols = slice(i * 128, (i + 1) * 128)
        hidden.append((jax.nn.silu(_dot(xn_b, ff_buf[0, :, cols]))
                       * _dot(xn_b, ff_buf[1, :, cols])).astype(_BF16))

    _wait_all(wd_buf, wd_sem)
    y = 0.0
    for i in _spread(pending[wd_done:], d_ff // 128):
        y = y + _dot(hidden[i], wd_buf[i * 128:(i + 1) * 128, :])
    gate_scr[...] = jax.nn.silu(xn + (xn * 0.0 + y * jax.nn.sigmoid(route)))

    def attend(step, carry, copies):
        b, g, c = split(step)
        slot = step % slots
        rows = pl.ds(b * _GROUP if isinstance(b, int) else pl.multiple_of(b * _GROUP, _GROUP),
                     _GROUP)
        m_prev, l_prev, acc = carry
        q = q_scr[g, rows, :].astype(_BF16)
        half = len(copies) // 8 * 4
        _wait_all(kv_buf.at[slot], kv_sem.at[slot])
        for j in _spread(copies[:half], _GROUP):
            s_j = jax.lax.dot_general(q, kv_buf[slot, 0, j], (((1,), (1,)), ((), ())),
                                      preferred_element_type=_F32)
            s = s_j if j == 0 else jnp.where(sublane(_GROUP, keys) == j, s_j, s)
        s = s * scale
        cols = [s[:, i:i + 128] for i in range(0, keys, 128)]
        m_new = jnp.maximum(
            m_prev, jnp.max(functools.reduce(jnp.maximum, cols), axis=-1, keepdims=True))
        alpha = jnp.exp(m_prev - m_new)
        cols = [jnp.exp(col - m_new) for col in cols]
        l_new = alpha * l_prev + functools.reduce(jnp.add, cols)
        p = jnp.concatenate(cols, axis=-1).astype(_BF16)
        for j in _spread(copies[half:], _GROUP):
            pv_j = _dot(p, kv_buf[slot, 1, j])
            pv = pv_j if j == 0 else jnp.where(sublane(_GROUP, _HEAD_DIM) == j, pv_j, pv)
        acc = alpha * acc + pv

        last = c == chunks - 1

        @pl.when(last)
        def _():
            o_scr[g, rows, :] = acc / jnp.sum(l_new, axis=-1, keepdims=True)

        return (jnp.where(last, -jnp.inf, m_new), jnp.where(last, 0.0, l_new),
                jnp.where(last, 0.0, acc))

    def main_step(step, carry):
        nxt = step + ahead
        return attend(step, carry, kv_copies(nxt, nxt % slots))

    carry = (jnp.full((_GROUP, _HEAD_DIM), -jnp.inf, _F32),
             jnp.zeros((_GROUP, _HEAD_DIM), _F32),
             jnp.zeros((_GROUP, _HEAD_DIM), _F32))
    carry = jax.lax.fori_loop(0, n_kv - ahead, main_step, carry)

    order = [h for i in range(4) for h in range(i, heads, 4)]
    wo_heads, wo_copies = [], []
    for i, size in enumerate(wo_groups):
        wo_heads.append(order[:size])
        order = order[size:]
        wo_copies += _copies(wo_hbm, wo_buf, wo_sem.at[i], [
            _tiles(h * _HEAD_DIM, (h + 1) * _HEAD_DIM, 16, d_model, d_model)
            for h in wo_heads[-1]])
    assert not order
    pending = _with_queues(wo_copies, 2)
    per_step = 2 * _GROUP * keys // piece
    for step in range(n_kv - ahead, n_kv):
        carry = attend(step, carry, pending[:per_step])
        pending = pending[per_step:]

    place = {head_of(g, j): (g, j) for g in range(groups) for j in range(_GROUP)}
    model_rows = sublane(batch * _GROUP, d_model)
    s = 0.0
    for i, batch_heads in enumerate(wo_heads):
        _wait_all(wo_buf.at[pl.ds(0, len(batch_heads) * _HEAD_DIM)], wo_sem.at[i])
        for n in _spread(pending, len(batch_heads)):
            h = batch_heads[n]
            g, j = place[h]
            s_h = _dot(o_scr[g].astype(_BF16), wo_buf[h * _HEAD_DIM:(h + 1) * _HEAD_DIM, :])
            s = s + jnp.where(model_rows == j, s_h, 0.0)
        pending = []
    update = jnp.concatenate(
        [jnp.sum(s[b * _GROUP:(b + 1) * _GROUP], axis=0, keepdims=True)
         * gate_scr[b * _GROUP:b * _GROUP + 1, :] for b in range(batch)], axis=0)
    out_buf[...] = (x_buf[...].astype(_F32) + update).astype(out_buf.dtype)
    out_copy = pltpu.make_async_copy(out_buf, out_hbm, x_sem)
    out_copy.start()
    out_copy.wait()


def _call(x, k, v, wq, wo, wr, wg, wu, wd, *, keys=256, piece=64, stride=2, slots=4,
          wo_groups=(8, 8, 8, 4, 2, 2), **params):
    batch, heads, seq, head_dim = k.shape
    d_model = x.shape[-1]
    assert head_dim == _HEAD_DIM and x.shape[1] == 1
    assert seq % keys == 0 and keys % piece == 0 and heads % (stride * _GROUP) == 0
    hbm = pl.BlockSpec(memory_space=pltpu.HBM)
    out = pl.pallas_call(
        functools.partial(_kernel, heads=heads, seq=seq, keys=keys, piece=piece, stride=stride,
                          slots=slots, wo_groups=wo_groups),
        in_specs=[hbm] * 9,
        out_specs=hbm,
        out_shape=jax.ShapeDtypeStruct((batch, d_model), x.dtype),
        scratch_shapes=[
            pltpu.VMEM((slots, 2, _GROUP, keys, head_dim), k.dtype),
            pltpu.VMEM(wq.shape, wq.dtype),
            pltpu.VMEM(wo.shape, wo.dtype),
            pltpu.VMEM((2,) + wg.shape, wg.dtype),
            pltpu.VMEM(wd.shape, wd.dtype),
            pltpu.VMEM((batch, d_model), x.dtype),
            pltpu.VMEM(wr.shape, wr.dtype),
            pltpu.VMEM((heads // _GROUP, batch * _GROUP, head_dim), _F32),
            pltpu.VMEM((heads // _GROUP, batch * _GROUP, head_dim), _F32),
            pltpu.VMEM((batch * _GROUP, d_model), _F32),
            pltpu.VMEM((batch, d_model), x.dtype),
            pltpu.SemaphoreType.DMA((5,)),
            pltpu.SemaphoreType.DMA((len(wo_groups),)),
            pltpu.SemaphoreType.DMA((slots,)),
        ],
        compiler_params=pltpu.CompilerParams(vmem_limit_bytes=64 * 1024 * 1024, **params),
    )(x.reshape(batch, d_model), k.reshape(-1, head_dim), v.reshape(-1, head_dim),
      wq, wo, wr, wg, wu, wd)
    return out.reshape(x.shape)


@jax.jit
def pallas_recurrent_scan__mha_block_cached__moe_arch_mod__decode_kernel(
    A_x: jax.Array,
    A_k_cache: jax.Array,
    A_v_cache: jax.Array,
    A_wq: jax.Array,
    A_wo: jax.Array,
    B_x: jax.Array,
    B_w_r: jax.Array,
    B_w_gate: jax.Array,
    B_w_up: jax.Array,
    B_w_down: jax.Array,
):
    del B_x
    return _call(A_x, A_k_cache, A_v_cache, A_wq, A_wo, B_w_r, B_w_gate, B_w_up, B_w_down)
```

```python
import functools

import jax
import jax.numpy as jnp
import jax.experimental.pallas as pl
import jax.experimental.pallas.tpu as pltpu

_HEAD_DIM = 128
_GROUP = 8
_LAG = 128
_EPS = 1e-5

_F32 = jnp.float32
_BF16 = jnp.bfloat16


def _dot(a, b):
    return jnp.dot(a, b, preferred_element_type=_F32)


def _tiles(r0, r1, rows, cols, width):
    return [(pl.ds(r, rows), pl.ds(c, width))
            for r in range(r0, r1, rows) for c in range(0, cols, width)]


def _bands(n_rows, n, *tile):
    return [_tiles(i * n_rows // n, (i + 1) * n_rows // n, *tile) for i in range(n)]


def _interleave(streams):
    return [item for group in zip(*streams, strict=True) for item in group]


def _copies(src, dst, sem, streams):
    return [(src.at[idx], dst.at[idx], sem) for idx in _interleave(streams)]


def _with_queues(copies, run):
    return [(copy, i // run % 2) for i, copy in enumerate(copies)]


def _start(copies):
    for copy, queue in copies:
        pltpu.make_async_copy(*copy).start(priority=queue)


def _spread(copies, n):
    done = 0
    for i in range(n):
        yield i
        upto = len(copies) if i == n - 1 else len(copies) // 4 * (i + 1) // n * 4
        _start(copies[done:upto])
        done = upto


def _wait_all(buf, sem):
    pltpu.make_async_copy(buf, buf, sem).wait()


def _kernel(x_hbm, k_hbm, v_hbm, wq_hbm, wo_hbm, wr_hbm, wg_hbm, wu_hbm, wd_hbm,
            out_hbm,
            kv_buf, wq_buf, wo_buf, ff_buf, wd_buf, x_buf, wr_buf,
            q_scr, o_scr, gate_scr, out_buf, sem, wo_sem, kv_sem,
            *, heads, seq, keys, piece, stride, slots, wo_batches):
    batch, d_model = x_hbm.shape
    d_ff = wg_hbm.shape[1]
    groups = heads // _GROUP
    chunks = seq // keys
    n_kv = batch * groups * chunks
    ahead = slots - 1
    scale = _HEAD_DIM ** -0.5
    x_sem, wr_sem, wq_sem, ff_sem, wd_sem = (sem.at[i] for i in range(5))

    def head_of(g, j):
        return g // stride * (stride * _GROUP) + g % stride + j * stride

    def split(step):
        return step // (groups * chunks), step // chunks % groups, step % chunks

    def kv_copies(step, slot):
        b, g, c = split(step)
        base = (b * heads + head_of(g, 0)) * seq + c * keys
        copies = []
        for r in range(0, keys, piece):
            for first in range(0, _GROUP, 2):
                for which, hbm in enumerate((k_hbm, v_hbm)):
                    for j in (first, first + 1):
                        src = base + head_of(0, j) * seq + r
                        if not isinstance(src, int):
                            src = pl.multiple_of(src, piece)
                        copies.append((hbm.at[pl.ds(src, piece)],
                                       kv_buf.at[slot, which, j, pl.ds(r, piece)],
                                       kv_sem.at[slot]))
        return _with_queues(copies, 2)

    def sublane(rows, cols):
        return jax.lax.broadcasted_iota(jnp.int32, (rows, cols), 0) % _GROUP

    wq_copies = _copies(wq_hbm, wq_buf, wq_sem, _bands(d_model, 8, 8, wq_hbm.shape[1], 1024))
    ff_copies = _interleave([
        _copies(wg_hbm, ff_buf.at[0], ff_sem, _bands(d_model, 4, 8, d_ff, d_ff)),
        _copies(wu_hbm, ff_buf.at[1], ff_sem, _bands(d_model, 4, 8, d_ff, d_ff))])
    wd_copies = _copies(wd_hbm, wd_buf, wd_sem, _bands(d_ff, 4, 16, d_model, d_model))
    pending = _with_queues(wq_copies, 2) + _with_queues(ff_copies, 1) + _with_queues(wd_copies, 2)
    for step in range(ahead):
        pending += kv_copies(step, step)
    wq_done = len(wq_copies) + _LAG
    ff_done = wq_done + len(ff_copies)
    wd_done = ff_done + len(wd_copies)

    _start(_with_queues([(x_hbm, x_buf, x_sem), (wr_hbm, wr_buf, wr_sem)], 1))
    _start(pending[:_LAG // 2])
    _wait_all(x_buf, x_sem)
    _wait_all(wr_buf, wr_sem)
    x = x_buf[...].astype(_F32)
    x = jnp.concatenate(
        [jnp.broadcast_to(x[b:b + 1], (_GROUP, d_model)) for b in range(batch)], axis=0)
    cent = x - jnp.mean(x, axis=-1, keepdims=True)
    var = jnp.mean(cent * cent, axis=-1, keepdims=True)
    xn_b = (cent / jnp.sqrt(var + _EPS)).astype(_BF16)
    xn = xn_b.astype(_F32)
    route = jnp.sum(xn * wr_buf[...].astype(_F32).reshape(1, d_model), axis=-1, keepdims=True)
    _start(pending[_LAG // 2:wq_done])

    _wait_all(wq_buf, wq_sem)
    head_rows = sublane(batch * _GROUP, _HEAD_DIM)
    for i in _spread(pending[wq_done:ff_done], heads):
        g, j = divmod(i, _GROUP)
        h = head_of(g, j)
        q_h = _dot(xn_b, wq_buf[:, h * _HEAD_DIM:(h + 1) * _HEAD_DIM])
        q = q_h if j == 0 else jnp.where(head_rows == j, q_h, q)
        if j == _GROUP - 1:
            q_scr[g] = q

    _wait_all(ff_buf, ff_sem)
    hidden = []
    for i in _spread(pending[ff_done:wd_done], d_ff // 128 * 2):
        cols = slice(i // 2 * 128, (i // 2 + 1) * 128)
        if i % 2 == 0:
            gate = jax.nn.silu(_dot(xn_b, ff_buf[0, :, cols]))
        else:
            hidden.append((gate * _dot(xn_b, ff_buf[1, :, cols])).astype(_BF16))

    _wait_all(wd_buf, wd_sem)
    y = 0.0
    for i in _spread(pending[wd_done:], d_ff // 128):
        y = y + _dot(hidden[i], wd_buf[i * 128:(i + 1) * 128, :])
    gate_scr[...] = jax.nn.silu(xn + (xn * 0.0 + y * jax.nn.sigmoid(route)))

    def attend(step, carry, copies):
        b, g, c = split(step)
        slot = step % slots
        rows = pl.ds(b * _GROUP if isinstance(b, int) else pl.multiple_of(b * _GROUP, _GROUP),
                     _GROUP)
        m_prev, l_prev, acc = carry
        q = q_scr[g, rows, :].astype(_BF16)
        half = len(copies) // 8 * 4
        _wait_all(kv_buf.at[slot], kv_sem.at[slot])
        for j in _spread(copies[:half], _GROUP):
            s_j = jax.lax.dot_general(q, kv_buf[slot, 0, j], (((1,), (1,)), ((), ())),
                                      preferred_element_type=_F32)
            s = s_j if j == 0 else jnp.where(sublane(_GROUP, keys) == j, s_j, s)
        s = s * scale
        cols = [s[:, i:i + 128] for i in range(0, keys, 128)]
        m_new = jnp.maximum(
            m_prev, jnp.max(functools.reduce(jnp.maximum, cols), axis=-1, keepdims=True))
        shift = jnp.where(m_new == -jnp.inf, 0.0, m_new)
        alpha = jnp.exp(m_prev - shift)
        cols = [jnp.exp(col - shift) for col in cols]
        l_new = alpha * l_prev + functools.reduce(jnp.add, cols)
        p = jnp.concatenate(cols, axis=-1).astype(_BF16)
        for j in _spread(copies[half:], _GROUP):
            pv_j = _dot(p, kv_buf[slot, 1, j])
            pv = pv_j if j == 0 else jnp.where(sublane(_GROUP, _HEAD_DIM) == j, pv_j, pv)
        acc = alpha * acc + pv

        last = c == chunks - 1

        @pl.when(last)
        def _():
            o_scr[g, rows, :] = acc / jnp.sum(l_new, axis=-1, keepdims=True)

        return (jnp.where(last, -jnp.inf, m_new), jnp.where(last, 0.0, l_new),
                jnp.where(last, 0.0, acc))

    def main_step(step, carry):
        nxt = step + ahead
        return attend(step, carry, kv_copies(nxt, nxt % slots))

    carry = (jnp.full((_GROUP, _HEAD_DIM), -jnp.inf, _F32),
             jnp.zeros((_GROUP, _HEAD_DIM), _F32),
             jnp.zeros((_GROUP, _HEAD_DIM), _F32))
    carry = jax.lax.fori_loop(0, n_kv - ahead, main_step, carry)

    order = [h for i in range(4) for h in range(i, heads, 4)]
    firsts = [sum(wo_batches[:i]) for i in range(len(wo_batches))]
    wo_copies = []
    for i, (first, size) in enumerate(zip(firsts, wo_batches)):
        wo_copies += _interleave([
            [(wo_hbm.at[pl.ds(order[n] * _HEAD_DIM + r, 16)], wo_buf.at[n, pl.ds(r, 16)],
              wo_sem.at[i]) for r in range(0, _HEAD_DIM, 16)]
            for n in range(first, first + size)])
    pending = _with_queues(wo_copies, 2)
    per_step = 2 * _GROUP * keys // piece
    for step in range(n_kv - ahead, n_kv):
        carry = attend(step, carry, pending[:per_step])
        pending = pending[per_step:]
    assert len(wo_copies) - len(pending) >= wo_batches[0] * _HEAD_DIM // 16

    place = {head_of(g, j): (g, j) for g in range(groups) for j in range(_GROUP)}
    model_rows = sublane(batch * _GROUP, d_model)
    s = 0.0
    for i, (first, size) in enumerate(zip(firsts, wo_batches)):
        _wait_all(wo_buf.at[pl.ds(first, size)], wo_sem.at[i])
        for n in _spread(pending, size):
            g, j = place[order[first + n]]
            s_h = _dot(o_scr[g].astype(_BF16), wo_buf[first + n])
            s = s + jnp.where(model_rows == j, s_h, 0.0)
        pending = []
    update = jnp.concatenate(
        [jnp.sum(s[b * _GROUP:(b + 1) * _GROUP], axis=0, keepdims=True)
         * gate_scr[b * _GROUP:b * _GROUP + 1, :] for b in range(batch)], axis=0)
    out_buf[...] = (x_buf[...].astype(_F32) + update).astype(out_buf.dtype)
    out_copy = pltpu.make_async_copy(out_buf, out_hbm, x_sem)
    out_copy.start()
    out_copy.wait()


def _call(x, k, v, wq, wo, wr, wg, wu, wd, *, keys=256, piece=64, stride=2, slots=4,
          wo_batches=(8, 8, 8, 4, 2, 2), interpret=False, **params):
    batch, heads, seq, head_dim = k.shape
    d_model = x.shape[-1]
    assert head_dim == _HEAD_DIM and x.shape[1] == 1
    assert seq % keys == 0 and keys % piece == 0 and heads % (stride * _GROUP) == 0
    assert sum(wo_batches) == heads
    hbm = pl.BlockSpec(memory_space=pltpu.HBM)
    out = pl.pallas_call(
        functools.partial(_kernel, heads=heads, seq=seq, keys=keys, piece=piece, stride=stride,
                          slots=slots, wo_batches=wo_batches),
        in_specs=[hbm] * 9,
        out_specs=hbm,
        out_shape=jax.ShapeDtypeStruct((batch, d_model), x.dtype),
        scratch_shapes=[
            pltpu.VMEM((slots, 2, _GROUP, keys, head_dim), k.dtype),
            pltpu.VMEM(wq.shape, wq.dtype),
            pltpu.VMEM((heads, head_dim, d_model), wo.dtype),
            pltpu.VMEM((2,) + wg.shape, wg.dtype),
            pltpu.VMEM(wd.shape, wd.dtype),
            pltpu.VMEM((batch, d_model), x.dtype),
            pltpu.VMEM(wr.shape, wr.dtype),
            pltpu.VMEM((heads // _GROUP, batch * _GROUP, head_dim), _F32),
            pltpu.VMEM((heads // _GROUP, batch * _GROUP, head_dim), _F32),
            pltpu.VMEM((batch * _GROUP, d_model), _F32),
            pltpu.VMEM((batch, d_model), x.dtype),
            pltpu.SemaphoreType.DMA((5,)),
            pltpu.SemaphoreType.DMA((len(wo_batches),)),
            pltpu.SemaphoreType.DMA((slots,)),
        ],
        compiler_params=pltpu.CompilerParams(vmem_limit_bytes=64 * 1024 * 1024, **params),
        interpret=interpret,
    )(x.reshape(batch, d_model), k.reshape(-1, head_dim), v.reshape(-1, head_dim),
      wq, wo, wr, wg, wu, wd)
    return out.reshape(x.shape)


@jax.jit
def pallas_recurrent_scan__mha_block_cached__moe_arch_mod__decode_kernel(
    A_x: jax.Array,
    A_k_cache: jax.Array,
    A_v_cache: jax.Array,
    A_wq: jax.Array,
    A_wo: jax.Array,
    B_x: jax.Array,
    B_w_r: jax.Array,
    B_w_gate: jax.Array,
    B_w_up: jax.Array,
    B_w_down: jax.Array,
):
    del B_x
    return _call(A_x, A_k_cache, A_v_cache, A_wq, A_wo, B_w_r, B_w_gate, B_w_up, B_w_down)
```
